```python
import os as _os
_os.environ.setdefault("JAX_PLATFORMS", "cpu")
import jax
import jax.numpy as jnp

def _softmax(x, axis=-1):
    return jax.nn.softmax(x, axis=axis)
def _gelu(x):
    return jax.nn.gelu(x, approximate=True)
def _silu(x):
    return jax.nn.silu(x)
def _sigmoid(x):
    return jax.nn.sigmoid(x)
def _layernorm(x, axis=-1, eps=1e-5):
    m = jnp.mean(x, axis=axis, keepdims=True)
    v = jnp.var(x, axis=axis, keepdims=True)
    return (x - m) / jnp.sqrt(v + eps)
def _scatter_add(tgt, idx, src, axis=0):
    return tgt.at[idx].add(src)
def _segment_sum(src, seg, n):
    return jax.ops.segment_sum(src, seg, n)
class _Rng:
    def __init__(self, key):
        self._k = key
    def _next(self):
        self._k, sub = jax.random.split(self._k)
        return sub
    def normal(self, shape):
        return jax.random.normal(self._next(), shape, dtype=jnp.bfloat16)
    def randint(self, lo, hi, shape):
        return jax.random.randint(self._next(), shape, lo, hi, dtype=jnp.int32)
    def uniform(self, shape, lo=0.0, hi=1.0):
        return jax.random.uniform(self._next(), shape, jnp.bfloat16, lo, hi)
    def permutation(self, n):
        return jax.random.permutation(self._next(), n)


kernel_name = 'standalone__gqa_block_cached__near_ridge'

def setup_inputs():
    _rng = _Rng(jax.random.key(int.from_bytes(__import__("os").urandom(4), "little")))
    _w = (lambda a: (lambda t: t.astype(jnp.bfloat16) if jnp.issubdtype(t.dtype, jnp.floating) else t)(jnp.asarray(a)))
    B, Sq, D = 8, 80, 512
    Hq, Hkv, Sk, Dh = 32, 8, 2048, 128
    assert Hq % Hkv == 0, (Hq, Hkv)
    return {
        "x": _w((lambda *s: _rng.normal(s) * 0.8)(B, Sq, D)),
        "k_cache": _w((lambda *s: _rng.normal(s) * 0.8)(B, Hkv, Sk, Dh)),
        "v_cache": _w((lambda *s: _rng.normal(s) * 0.05)(B, Hkv, Sk, Dh)),
        "wq": _w((lambda *s: _rng.normal(s) * 0.8)(D, Hq * Dh) * (D ** -0.5)),
        "wo": _w((lambda *s: _rng.normal(s) * 0.05)(Hq * Dh, D) * ((Hq * Dh) ** -0.5)),
    }

def reference(x, k_cache, v_cache, wq, wo):
    B, Sq, D = x.shape
    Hq, Dh = 32, 128
    Hkv = k_cache.shape[1]
    rep = Hq // Hkv
    q = (lambda x, *d: x.transpose(*d))((x @ wq).reshape(B, Sq, Hq, Dh), 0, 2, 1, 3)
    k = jnp.repeat(k_cache, rep, axis=1)
    v = jnp.repeat(v_cache, rep, axis=1)
    scores = jnp.einsum("bhqd,bhkd->bhqk", q, k) * (Dh ** -0.5)
    p = _softmax(scores, axis=-1)
    o = jnp.einsum("bhqk,bhkd->bhqd", p, v)
    return (lambda x, *d: x.transpose(*d))(o, 0, 2, 1, 3).reshape(B, Sq, Hq * Dh) @ wo
```

```python
import functools
import math
import jax
import jax.numpy as jnp
from jax import lax
import jax.experimental.pallas as pl
import jax.experimental.pallas.tpu as pltpu

HQ = 32
DH = 128
TK = 512
U = 4
SCOPES = 0
CG = 2


def _kernel(x_hbm, k_hbm, v_hbm, wq_hbm, wo_hbm, out_hbm,
            x_s, wq_s, wo_s, kv_s, q_scr, s_scr, m_scr, o_scr, acc_scr, out_s,
            kv_sem, wq_sem, wo_sem, p_sem, o_sem, *, B, Sq, rep, Hkv, Sk):
    NS = B * Hkv // U
    BU = B // U
    scale = (DH ** -0.5) * math.log2(math.e)
    R = rep * Sq
    nC = Sk // TK
    nt = TK // 128
    logBU = BU.bit_length() - 1
    D = x_s.shape[-1]
    G = rep * DH
    PR = D // BU
    assert D == G

    def gb(t):
        if isinstance(t, int):
            return t >> logBU, t & (BU - 1)
        return lax.shift_right_logical(t, logBU), t & (BU - 1)

    def mult(v, m):
        return v * m if isinstance(v, int) else pl.multiple_of(v * m, m)

    def wait(c, name):
        if SCOPES:
            with jax.named_scope(name):
                c.wait()
        else:
            c.wait()

    def k_copy(t, sem=None):
        g, bb = gb(t)
        slot = t & 1
        return pltpu.make_async_copy(k_hbm.at[pl.ds(bb * U, U), g], kv_s.at[slot, 0],
                                     kv_sem.at[slot] if sem is None else sem)

    def v_copy(t, sem=None):
        g, bb = gb(t)
        slot = (t + 1) & 1
        return pltpu.make_async_copy(v_hbm.at[pl.ds(bb * U, U), g], kv_s.at[slot, 1],
                                     kv_sem.at[slot] if sem is None else sem)

    def kv_wait(i):
        slot = i & 1
        wait(pltpu.make_async_copy(kv_s.at[slot], kv_s.at[slot], kv_sem.at[slot]), "kv_wait")

    _next_sem = [0]

    def new_sem():
        s = p_sem.at[_next_sem[0]]
        _next_sem[0] += 1
        return s

    def k_items(t, u0, n):
        g, bb = gb(t)
        return pltpu.make_async_copy(k_hbm.at[pl.ds(bb * U + u0, n), g],
                                     kv_s.at[t & 1, 0, pl.ds(u0, n)], new_sem())

    def v_items(t, u0, n):
        g, bb = gb(t)
        return pltpu.make_async_copy(v_hbm.at[pl.ds(bb * U + u0, n), g],
                                     kv_s.at[(t + 1) & 1, 1, pl.ds(u0, n)], new_sem())

    def wq_piece(n):
        g, pc = gb(n)
        gs = g & (Hkv - 1)
        return pltpu.make_async_copy(wq_hbm.at[pl.ds(mult(pc, PR), PR), pl.ds(mult(gs, G), G)],
                                     wq_s.at[g, pl.ds(mult(pc, PR), PR), :], wq_sem.at[0])

    def wo_piece(n):
        g, pc = gb(n)
        ns = n & (NS - 1)
        return pltpu.make_async_copy(wo_hbm.at[pl.ds(mult(ns, PR), PR), :],
                                     wo_s.at[g, pl.ds(mult(pc, PR), PR), :], wo_sem.at[0])

    def qproj(t):
        g, bb = gb(t)
        q = jnp.dot(x_s[bb], wq_s[g], preferred_element_type=jnp.float32) * scale
        q = q.astype(jnp.bfloat16)
        for u in range(U):
            for h in range(rep):
                q_scr[u, h * Sq:(h + 1) * Sq, :] = q[u * Sq:(u + 1) * Sq, h * DH:(h + 1) * DH]

    def qk(u, slot):
        q = q_scr[u]
        pmx = None
        for j in range(nC):
            s = lax.dot_general(q, kv_s[slot, 0, u, j * TK:(j + 1) * TK, :], (((1,), (1,)), ((), ())),
                                preferred_element_type=jnp.float32)
            s_scr[u, :, j * TK:(j + 1) * TK] = s
            pm = s[:, 0:128]
            for t in range(1, nt):
                pm = jnp.maximum(pm, s[:, t * 128:(t + 1) * 128])
            pmx = pm if pmx is None else jnp.maximum(pmx, pm)
        m_scr[u] = jnp.broadcast_to(jnp.max(pmx, axis=-1, keepdims=True), (R, 128))

    def pv(u, slot):
        m = m_scr[u]
        p = jnp.exp2(s_scr[u] - jnp.concatenate([m] * (Sk // 128), axis=1))
        lp = None
        for j in range(nC):
            ps = p[:, j * TK:j * TK + 128]
            for t in range(1, nt):
                ps = ps + p[:, j * TK + t * 128:j * TK + (t + 1) * 128]
            lp = ps if lp is None else lp + ps
        acc = jnp.dot(p.astype(jnp.bfloat16), kv_s[slot, 1, u], preferred_element_type=jnp.float32)
        l = jnp.sum(lp, axis=-1, keepdims=True)
        r = pl.reciprocal(l, approx=True)
        r = r * (2.0 - l * r)
        o = (acc * r).astype(jnp.bfloat16)
        for h in range(rep):
            o_scr[u * Sq:(u + 1) * Sq, h * DH:(h + 1) * DH] = o[h * Sq:(h + 1) * Sq, :]

    def oproj(t):
        g, bb = gb(t)
        y = jnp.dot(o_scr[...], wo_s[g], preferred_element_type=jnp.float32)
        if isinstance(g, int):
            if g > 0:
                y = y + acc_scr[bb]
        else:
            y = y + jnp.where(g > 0, acc_scr[bb], 0.0)
        acc_scr[bb] = y
        out_s[bb] = y.astype(out_s.dtype)

    WQ_OFF = BU + 1
    WO_OFF = BU - 2

    def x_copy(bb):
        return pltpu.make_async_copy(x_hbm.at[bb], x_s.at[bb], new_sem())

    def wq_bulk(n0, n1):
        g, pc = gb(n0)
        assert gb(n1 - 1)[0] == g
        rows = pl.ds(pc * PR, (n1 - n0) * PR)
        return pltpu.make_async_copy(wq_hbm.at[rows, pl.ds(g * G, G)], wq_s.at[g, rows, :], new_sem())

    xs = [x_copy(bb) for bb in range(BU)]
    wq0 = wq_bulk(0, BU)
    k0 = [k_items(0, u, 1) for u in range(U)]
    v0 = [v_items(0, u, CG) for u in range(0, U, CG)]
    k1 = k_copy(1, new_sem())
    v1 = v_copy(1, new_sem())
    k2 = k_copy(2, new_sem())
    wo0 = pltpu.make_async_copy(wo_hbm.at[pl.ds(0, G), :], wo_s.at[0], new_sem())
    last = 1 + WQ_OFF
    wq1 = wq_bulk(BU, min(last + 1, 2 * BU))
    wq2 = wq_bulk(2 * BU, last + 1) if last + 1 > 2 * BU else None

    first = [xs[0], wq0] + k0 + [xs[1]] + v0 + [k1]
    if BU > 2:
        first += [xs[2], wo0, v1]
    else:
        first += [wq1, wo0, v1]
    for c in first:
        c.start()

    wait(xs[0], "w_x0")
    wait(wq0, "w_wq0")
    qproj(0)
    for u in range(U):
        wait(k0[u], "w_k0")
        if u == U - 1:
            wait(xs[1], "w_x1")
        qk(u, 0)
    qproj(1)

    k2.start()
    for bb in range(3, BU):
        xs[bb].start()
    for c in range(len(v0)):
        wait(v0[c], "w_v0")
        for u in range(c * CG, (c + 1) * CG):
            pv(u, 1)
    v_copy(2).start()
    wait(k1, "w_k1")
    wait(xs[2] if BU > 2 else wq1, "w_x2")
    for u in range(U):
        qk(u, 1)
    qproj(2)

    k_copy(3).start()
    (wq1 if BU > 2 else wq2).start()
    wq_piece(2 + WQ_OFF).start()
    wo_piece(2 + WO_OFF).start()
    wait(wo0, "w_wo0")
    wait(v1, "w_v1")
    oproj(0)
    for u in range(U):
        pv(u, 0)
    wait(k2, "w_k2")
    for bb in range(3, BU):
        wait(xs[bb], "w_x3")
    for u in range(U):
        qk(u, 0)
    qproj(3)
    wait(wq1 if BU > 2 else wq2, "w_wq1")

    def body(i, carry):
        slot = i & 1
        kv_wait(i)
        wq_piece(i - 1 + WQ_OFF).wait()
        wo_piece(i - 1 + WO_OFF).wait()
        v_copy(i).start()
        k_copy(i + 1).start()
        wq_piece(i + WQ_OFF).start()
        oproj(i - 2)
        wo_piece(i + WO_OFF).start()
        for u in range(U):
            pv(u, slot)
        for u in range(U):
            qk(u, slot)
        qproj(i + 1)
        return carry

    lax.fori_loop(3, NS - 1, body, 0)

    def out_copy(bb):
        return pltpu.make_async_copy(out_s.at[bb], out_hbm.at[bb], o_sem.at[bb])

    i = NS - 1
    vl = v_copy(i, new_sem())
    kv_wait(i)
    wq_piece(i - 1 + WQ_OFF).wait()
    wo_piece(i - 1 + WO_OFF).wait()
    vl.start()
    if WO_OFF == 0:
        wol = wo_piece(i)
    oproj(i - 2)
    if WO_OFF == 0:
        wol.start()
    for u in range(U):
        pv(u, i & 1)
    for u in range(U):
        qk(u, i & 1)

    for bb in range(BU - 2):
        out_copy(bb).start()
    if WO_OFF == 0:
        wol.wait()
    wait(vl, "w_vl")
    oproj(NS - 2)
    out_copy(BU - 2).start()
    for u in range(U):
        pv(u, NS & 1)
    oproj(NS - 1)
    out_copy(BU - 1).start()
    for bb in range(BU):
        wait(out_copy(bb), "w_out")


@jax.jit
def pallas_standalone__gqa_block_cached__near_ridge_kernel(x, k_cache, v_cache, wq, wo):
    B, Sq, D = x.shape
    _, Hkv, Sk, Dh = k_cache.shape
    rep = HQ // Hkv
    G = rep * Dh
    R = rep * Sq
    BU = B // U
    assert BU & (BU - 1) == 0 and BU >= 2 and Hkv & (Hkv - 1) == 0
    kern = functools.partial(_kernel, B=B, Sq=Sq, rep=rep, Hkv=Hkv, Sk=Sk)
    any_spec = pl.BlockSpec(memory_space=pl.ANY)
    out = pl.pallas_call(
        kern,
        in_specs=[any_spec] * 5,
        out_specs=any_spec,
        out_shape=jax.ShapeDtypeStruct((BU, U * Sq, D), x.dtype),
        scratch_shapes=[
            pltpu.VMEM((BU, U * Sq, D), jnp.bfloat16),
            pltpu.VMEM((Hkv + 1, D, G), jnp.bfloat16),
            pltpu.VMEM((Hkv + 1, G, D), jnp.bfloat16),
            pltpu.VMEM((2, 2, U, Sk, Dh), jnp.bfloat16),
            pltpu.VMEM((U, R, Dh), jnp.bfloat16),
            pltpu.VMEM((U, R, Sk), jnp.float32),
            pltpu.VMEM((U, R, 128), jnp.float32),
            pltpu.VMEM((U * Sq, G), jnp.bfloat16),
            pltpu.VMEM((BU, U * Sq, D), jnp.float32),
            pltpu.VMEM((BU, U * Sq, D), jnp.bfloat16),
            pltpu.SemaphoreType.DMA((2,)),
            pltpu.SemaphoreType.DMA((1,)),
            pltpu.SemaphoreType.DMA((1,)),
            pltpu.SemaphoreType.DMA((10 + BU + 2 * U,)),
            pltpu.SemaphoreType.DMA((BU,)),
        ],
        compiler_params=pltpu.CompilerParams(
            vmem_limit_bytes=100 * 1024 * 1024,
            disable_bounds_checks=True,
        ),
    )(x.reshape(BU, U * Sq, D), k_cache, v_cache, wq, wo)
    return out.reshape(B, Sq, D)
```

```python
import functools
import math
import jax
import jax.numpy as jnp
from jax import lax
import jax.experimental.pallas as pl
import jax.experimental.pallas.tpu as pltpu

HQ = 32
DH = 128
TK = 512
SCOPES = 0
NOSEM = 1
XB0 = 2
NLQ = 2
X1N = 3
X1Q = 2


def _kernel(x_hbm, k_hbm, v_hbm, wq_hbm, wo_hbm, out_hbm,
            x_s, wq_s, wo_s, kv_s, q_all, s_scr, m_scr, o_scr, acc_scr, out_s, z_ref,
            sems, *, B, Sq, rep, Hkv, Sk):
    scale = (DH ** -0.5) * math.log2(math.e)
    R = rep * Sq
    nC = Sk // TK
    nt = TK // 128
    D = x_s.shape[-1]
    G = rep * DH

    def mult(v, m):
        return v * m if isinstance(v, int) else pl.multiple_of(v * m, m)

    def wait(c, name):
        if SCOPES:
            with jax.named_scope(name):
                c.wait()
        else:
            c.wait()

    def kv_sem(slot):
        return sems.at[slot]

    wo_sem = sems.at[2]
    _next_sem = [3 + Hkv]

    def new_sem():
        s = sems.at[_next_sem[0]]
        _next_sem[0] += 1
        return s

    def k_copy(g, sem, b0=0, n=B):
        return pltpu.make_async_copy(k_hbm.at[pl.ds(b0, n), g], kv_s.at[g & 1, 0, pl.ds(b0, n)], sem)

    def v_copy(g, sem, b0=0, n=B - 1):
        return pltpu.make_async_copy(v_hbm.at[pl.ds(b0, n), g], kv_s.at[g & 1, 1, pl.ds(b0 + 1, n)], sem)

    def vlast_copy(g, sem):
        return pltpu.make_async_copy(v_hbm.at[B - 1, g], kv_s.at[(g + 1) & 1, 1, 0], sem)

    def wq_copy(g):
        return pltpu.make_async_copy(wq_hbm.at[:, pl.ds(mult(g, G), G)], wq_s.at[g], sems.at[3 + g])

    def wo_copy(g, sem):
        return pltpu.make_async_copy(wo_hbm.at[pl.ds(mult(g, G), G), :], wo_s.at[g], sem)

    def x_copy(b0, n):
        rows = pl.ds(b0 * Sq, n * Sq)
        return pltpu.make_async_copy(x_hbm.at[rows], x_s.at[rows], new_sem())

    def out_copy(b0, n):
        return pltpu.make_async_copy(out_s.at[pl.ds(b0, n)], out_hbm.at[pl.ds(b0, n)], new_sem())

    def qproj(g, b0=0, nb=B):
        q = jnp.dot(x_s[b0 * Sq:(b0 + nb) * Sq, :], wq_s[g], preferred_element_type=jnp.float32) * scale
        q = q.astype(jnp.bfloat16)
        for u in range(nb):
            for h in range(rep):
                q_all[g, b0 + u, h * Sq:(h + 1) * Sq, :] = q[u * Sq:(u + 1) * Sq, h * DH:(h + 1) * DH]

    def qk(g, b):
        q = q_all[g, b]
        slot = g & 1
        pmx = None
        for j in range(nC):
            s = lax.dot_general(q, kv_s[slot, 0, b, j * TK:(j + 1) * TK, :], (((1,), (1,)), ((), ())),
                                preferred_element_type=jnp.float32)
            s_scr[0, :, j * TK:(j + 1) * TK] = s
            pm = s[:, 0:128]
            for t in range(1, nt):
                pm = jnp.maximum(pm, s[:, t * 128:(t + 1) * 128])
            pmx = pm if pmx is None else jnp.maximum(pmx, pm)
        m_scr[0] = jnp.broadcast_to(jnp.max(pmx, axis=-1, keepdims=True), (R, 128))

    def pv(slot, j0, tie=True):
        z = z_ref[0]
        m = m_scr[z]
        p = jnp.exp2(s_scr[z] - jnp.concatenate([m] * (Sk // 128), axis=1))
        lp = None
        for j in range(nC):
            ps = p[:, j * TK:j * TK + 128]
            for t in range(1, nt):
                ps = ps + p[:, j * TK + t * 128:j * TK + (t + 1) * 128]
            lp = ps if lp is None else lp + ps
        acc = jnp.dot(p.astype(jnp.bfloat16), kv_s[slot, 1, j0], preferred_element_type=jnp.float32)
        if tie:
            lp = jnp.where(z != 0, acc, lp)
        l = jnp.sum(lp, axis=-1, keepdims=True)
        r = pl.reciprocal(l, approx=True)
        r = r * (2.0 - l * r)
        o = (acc * r).astype(jnp.bfloat16)
        for h in range(rep):
            o_scr[0, :, h * DH:(h + 1) * DH] = o[h * Sq:(h + 1) * Sq, :]

    def oproj(g, b, maybe_first=False):
        y = jnp.dot(o_scr[z_ref[0]], wo_s[g], preferred_element_type=jnp.float32)
        static = isinstance(g, int)
        if static:
            if g > 0:
                y = y + acc_scr[b]
        elif maybe_first:
            y = y + jnp.where(g > 0, acc_scr[b], 0.0)
        else:
            y = y + acc_scr[b]
        if not (static and g == Hkv - 1):
            acc_scr[b] = y
        if not (static and g < Hkv - 1) and not maybe_first:
            out_s[b] = y.astype(out_s.dtype)

    def zstep(g, b):
        pv(g & 1, b)
        qk(g, b)
        if b == 0:
            oproj(g - 1, B - 1, maybe_first=True)
        else:
            oproj(g, b - 1)

    def whole(_it, _carry):
        g1 = 1 + 2 * NLQ
        g2 = g1 + X1Q
        xa = x_copy(0, XB0)
        xb = x_copy(XB0, B - XB0)
        k0a = k_copy(0, new_sem(), 0, X1N)
        v0a = v_copy(0, new_sem(), 0, X1N - 1)
        wo0 = wo_copy(0, new_sem())
        v0b = v_copy(0, new_sem(), X1N - 1, B - X1N)
        k0b = k_copy(0, new_sem(), X1N, B - X1N)
        order = ([xa, wq_copy(0), xb] + [wq_copy(g) for g in range(1, g2)] + [k0a, v0a, wo0]
                 + [wq_copy(g) for g in range(g2, Hkv)] + [v0b, k0b]
                 + [vlast_copy(0, kv_sem(1)), k_copy(1, kv_sem(1)), v_copy(1, kv_sem(1)), wo_copy(1, wo_sem)])
        for c in order:
            c.start()

        wait(xa, "w_xa")
        wait(wq_copy(0), "w_wq0")
        qproj(0, 0, XB0)
        wait(xb, "w_xb")
        qproj(0, XB0, B - XB0)

        def qbody(j, carry):
            g = 2 * j + 1
            wait(wq_copy(g), "w_wq")
            wait(wq_copy(g + 1), "w_wq")
            qproj(g)
            qproj(g + 1)
            return carry

        lax.fori_loop(0, NLQ, qbody, 0)

        for c in [wq_copy(g) for g in range(g1, g2)] + [k0a, v0a, wo0]:
            wait(c, "w_x1")
        qk(0, 0)
        for g in range(g1, g2):
            qproj(g)
        for b in range(1, X1N):
            zstep(0, b)
        for c in [wq_copy(g) for g in range(g2, Hkv)] + [v0b, k0b]:
            wait(c, "w_x2")
        for g in range(g2, Hkv):
            qproj(g)
        for b in range(X1N, B):
            zstep(0, b)

        def body(g, carry):
            slot = g & 1
            wait(pltpu.make_async_copy(kv_s.at[slot], kv_s.at[slot], kv_sem(slot)), "kv_wait")
            wo_copy(g, wo_sem).wait()
            zstep(g, 0)
            vlast_copy(g, kv_sem(1 - slot)).start()

            @pl.when(g < Hkv - 1)
            def _():
                k_copy(g + 1, kv_sem(1 - slot)).start()
                v_copy(g + 1, kv_sem(1 - slot)).start()
                wo_copy(g + 1, wo_sem).start()

            for b in range(1, B):
                zstep(g, b)
            return carry

        lax.fori_loop(1, Hkv, body, 0)

        oa = out_copy(0, B - 1)
        ob = out_copy(B - 1, 1)
        oa.start()
        wait(vlast_copy(Hkv - 1, kv_sem(Hkv & 1)), "w_vl")
        pv(Hkv & 1, 0, tie=False)
        oproj(Hkv - 1, B - 1)
        ob.start()
        wait(oa, "w_out")
        wait(ob, "w_out")
        return _carry

    z_ref[0] = 0
    lax.fori_loop(0, 1 + z_ref[0], whole, 0)


@jax.jit
def pallas_standalone__gqa_block_cached__near_ridge_kernel(x, k_cache, v_cache, wq, wo):
    B, Sq, D = x.shape
    _, Hkv, Sk, Dh = k_cache.shape
    rep = HQ // Hkv
    G = rep * Dh
    R = rep * Sq
    kern = functools.partial(_kernel, B=B, Sq=Sq, rep=rep, Hkv=Hkv, Sk=Sk)
    any_spec = pl.BlockSpec(memory_space=pl.ANY)
    return pl.pallas_call(
        kern,
        in_specs=[any_spec] * 5,
        out_specs=any_spec,
        out_shape=jax.ShapeDtypeStruct((B, Sq, D), x.dtype),
        scratch_shapes=[
            pltpu.VMEM((B * Sq, D), jnp.bfloat16),
            pltpu.VMEM((Hkv, D, G), jnp.bfloat16),
            pltpu.VMEM((Hkv, G, D), jnp.bfloat16),
            pltpu.VMEM((2, 2, B, Sk, Dh), jnp.bfloat16),
            pltpu.VMEM((Hkv, B, R, Dh), jnp.bfloat16),
            pltpu.VMEM((1, R, Sk), jnp.float32),
            pltpu.VMEM((1, R, 128), jnp.float32),
            pltpu.VMEM((1, Sq, G), jnp.bfloat16),
            pltpu.VMEM((B, Sq, D), jnp.float32),
            pltpu.VMEM((B, Sq, D), jnp.bfloat16),
            pltpu.SMEM((1,), jnp.int32),
            pltpu.SemaphoreType.DMA((3 + Hkv + 9,)),
        ],
        compiler_params=pltpu.CompilerParams(
            vmem_limit_bytes=100 * 1024 * 1024,
            disable_bounds_checks=True,
            disable_semaphore_checks=bool(NOSEM),
        ),
    )(x.reshape(B * Sq, D), k_cache, v_cache, wq, wo)
```

```python
import functools
import math

import jax
import jax.numpy as jnp
from jax import lax
import jax.experimental.pallas as pl
import jax.experimental.pallas.tpu as pltpu

HQ = 32
DH = 128
TK = 512
XB0 = 2
NLQ = 2
X1N = 3
X1Q = 2


def _kernel(x_hbm, k_hbm, v_hbm, wq_hbm, wo_hbm, out_hbm,
            x_s, wq_s, wo_s, kv_s, q_all, s_scr, m_scr, o_scr, o2_scr, acc_scr, out_s, z_ref,
            sems, *, B, Sq, rep, Hkv, Sk):
    scale = (DH ** -0.5) * math.log2(math.e)
    R = rep * Sq
    nC = Sk // TK
    nt = TK // 128
    G = rep * DH

    def mult(v, m):
        return v * m if isinstance(v, int) else pl.multiple_of(v * m, m)

    def kv_sem(slot):
        return sems.at[slot]

    wo_sem = sems.at[2]
    next_sem = [3 + Hkv]

    def new_sem():
        s = sems.at[next_sem[0]]
        next_sem[0] += 1
        return s

    def k_copy(g, sem, b0=0, n=B):
        return pltpu.make_async_copy(k_hbm.at[pl.ds(b0, n), g], kv_s.at[g & 1, 0, pl.ds(b0, n)], sem)

    def v_copy(g, sem, b0=0, n=B - 1):
        return pltpu.make_async_copy(v_hbm.at[pl.ds(b0, n), g], kv_s.at[g & 1, 1, pl.ds(b0 + 1, n)], sem)

    def vlast_copy(g, sem):
        return pltpu.make_async_copy(v_hbm.at[B - 1, g], kv_s.at[(g + 1) & 1, 1, 0], sem)

    def wq_copy(g):
        return pltpu.make_async_copy(wq_hbm.at[:, pl.ds(mult(g, G), G)], wq_s.at[g], sems.at[3 + g])

    def wo_copy(g, sem):
        return pltpu.make_async_copy(wo_hbm.at[pl.ds(mult(g, G), G), :], wo_s.at[g], sem)

    def x_copy(b0, n):
        rows = pl.ds(b0 * Sq, n * Sq)
        return pltpu.make_async_copy(x_hbm.at[rows], x_s.at[rows], new_sem())

    def out_copy(b0, n):
        return pltpu.make_async_copy(out_s.at[pl.ds(b0, n)], out_hbm.at[pl.ds(b0, n)], new_sem())

    def qproj(g, b0=0, nb=B):
        q = jnp.dot(x_s[b0 * Sq:(b0 + nb) * Sq, :], wq_s[g], preferred_element_type=jnp.float32)
        q = q.astype(jnp.bfloat16)
        for u in range(nb):
            for h in range(rep):
                q_all[g, b0 + u, h * Sq:(h + 1) * Sq, :] = q[u * Sq:(u + 1) * Sq, h * DH:(h + 1) * DH]

    def qk(g, b):
        q = q_all[g, b]
        slot = g & 1
        pmx = None
        for j in range(nC):
            s = lax.dot_general(q, kv_s[slot, 0, b, j * TK:(j + 1) * TK, :], (((1,), (1,)), ((), ())),
                                preferred_element_type=jnp.float32) * scale
            s_scr[0, :, j * TK:(j + 1) * TK] = s
            pm = s[:, 0:128]
            for t in range(1, nt):
                pm = jnp.maximum(pm, s[:, t * 128:(t + 1) * 128])
            pmx = pm if pmx is None else jnp.maximum(pmx, pm)
        m_scr[0] = jnp.broadcast_to(jnp.max(pmx, axis=-1, keepdims=True), (R, 128))

    def pv(slot, j0, tie=True, h0=0, nh=rep, o_dst=o_scr):
        z = z_ref[0]
        rows = slice(h0 * Sq, (h0 + nh) * Sq)
        m = m_scr[z, rows, :]
        p = jnp.exp2(s_scr[z, rows, :] - jnp.concatenate([m] * (Sk // 128), axis=1))
        lp = None
        for j in range(nC):
            ps = p[:, j * TK:j * TK + 128]
            for t in range(1, nt):
                ps = ps + p[:, j * TK + t * 128:j * TK + (t + 1) * 128]
            lp = ps if lp is None else lp + ps
        acc = jnp.dot(p.astype(jnp.bfloat16), kv_s[slot, 1, j0], preferred_element_type=jnp.float32)
        if tie:
            lp = jnp.where(z != 0, acc, lp)
        l = jnp.sum(lp, axis=-1, keepdims=True)
        r = pl.reciprocal(l, approx=True)
        r = r * (2.0 - l * r)
        o = (acc * r).astype(jnp.bfloat16)
        for h in range(nh):
            o_dst[0, :, (h0 + h) * DH:(h0 + h + 1) * DH] = o[h * Sq:(h + 1) * Sq, :]

    def oproj(g, b, maybe_first=False):
        y = jnp.dot(o_scr[z_ref[0]], wo_s[g], preferred_element_type=jnp.float32)
        static = isinstance(g, int)
        if static:
            if g > 0:
                y = y + acc_scr[b]
        elif maybe_first:
            y = y + jnp.where(g > 0, acc_scr[b], 0.0)
        else:
            y = y + acc_scr[b]
        acc_scr[b] = y
        if not static and not maybe_first:
            out_s[b] = y.astype(out_s.dtype)

    def zstep(g, b):
        pv(g & 1, b)
        qk(g, b)
        if b == 0:
            oproj(g - 1, B - 1, maybe_first=True)
        else:
            oproj(g, b - 1)

    def whole(_, carry0):
        g1 = 1 + 2 * NLQ
        g2 = g1 + X1Q
        xa = x_copy(0, XB0)
        xb = x_copy(XB0, B - XB0)
        k0a = k_copy(0, new_sem(), 0, X1N)
        v0a = v_copy(0, new_sem(), 0, X1N - 1)
        wo0 = wo_copy(0, new_sem())
        v0b = v_copy(0, new_sem(), X1N - 1, B - X1N)
        k0b = k_copy(0, new_sem(), X1N, B - X1N)
        order = ([xa, wq_copy(0), xb] + [wq_copy(g) for g in range(1, g2)] + [k0a, v0a, wo0]
                 + [wq_copy(g) for g in range(g2, Hkv)] + [v0b, k0b]
                 + [vlast_copy(0, kv_sem(1)), k_copy(1, kv_sem(1)), v_copy(1, kv_sem(1)),
                    wo_copy(1, wo_sem)])
        for c in order:
            c.start()

        xa.wait()
        wq_copy(0).wait()
        qproj(0, 0, XB0)
        xb.wait()
        qproj(0, XB0, B - XB0)

        def qbody(j, carry):
            g = 2 * j + 1
            wq_copy(g).wait()
            wq_copy(g + 1).wait()
            qproj(g)
            qproj(g + 1)
            return carry

        lax.fori_loop(0, NLQ, qbody, 0)

        for c in [wq_copy(g) for g in range(g1, g2)] + [k0a, v0a, wo0]:
            c.wait()
        qk(0, 0)
        for g in range(g1, g2):
            qproj(g)
        for b in range(1, X1N):
            zstep(0, b)
        for c in [wq_copy(g) for g in range(g2, Hkv)] + [v0b, k0b]:
            c.wait()
        for g in range(g2, Hkv):
            qproj(g)
        for b in range(X1N, B):
            zstep(0, b)

        def body(g, carry):
            slot = g & 1
            pltpu.make_async_copy(kv_s.at[slot], kv_s.at[slot], kv_sem(slot)).wait()
            wo_copy(g, wo_sem).wait()
            zstep(g, 0)
            vlast_copy(g, kv_sem(1 - slot)).start()

            @pl.when(g < Hkv - 1)
            def _():
                k_copy(g + 1, kv_sem(1 - slot)).start()
                v_copy(g + 1, kv_sem(1 - slot)).start()
                wo_copy(g + 1, wo_sem).start()

            for b in range(1, B):
                zstep(g, b)
            return carry

        lax.fori_loop(1, Hkv, body, 0)

        oa = out_copy(0, B - 1)
        ob = out_copy(B - 1, 1)
        oa.start()
        vlast_copy(Hkv - 1, kv_sem(Hkv & 1)).wait()
        hh = rep // 2
        pv(Hkv & 1, 0, False, 0, hh, o_scr)
        pv(Hkv & 1, 0, False, hh, rep - hh, o2_scr)
        z = z_ref[0]
        y = acc_scr[B - 1] + jnp.dot(o_scr[z, :, :hh * DH], wo_s[Hkv - 1, :hh * DH, :],
                                     preferred_element_type=jnp.float32)
        y = y + jnp.dot(o2_scr[z, :, hh * DH:], wo_s[Hkv - 1, hh * DH:, :],
                        preferred_element_type=jnp.float32)
        out_s[B - 1] = y.astype(out_s.dtype)
        ob.start()
        oa.wait()
        ob.wait()
        return carry0

    z_ref[0] = 0
    lax.fori_loop(0, 1 + z_ref[0], whole, 0)


@jax.jit
def pallas_standalone__gqa_block_cached__near_ridge_kernel(x, k_cache, v_cache, wq, wo):
    B, Sq, D = x.shape
    _, Hkv, Sk, Dh = k_cache.shape
    rep = HQ // Hkv
    G = rep * Dh
    R = rep * Sq
    assert Dh == DH and Sk % TK == 0 and Sq % 16 == 0 and 1 + 2 * NLQ + X1Q <= Hkv and X1N < B
    kern = functools.partial(_kernel, B=B, Sq=Sq, rep=rep, Hkv=Hkv, Sk=Sk)
    any_spec = pl.BlockSpec(memory_space=pl.ANY)
    return pl.pallas_call(
        kern,
        in_specs=[any_spec] * 5,
        out_specs=any_spec,
        out_shape=jax.ShapeDtypeStruct((B, Sq, D), x.dtype),
        scratch_shapes=[
            pltpu.VMEM((B * Sq, D), jnp.bfloat16),
            pltpu.VMEM((Hkv, D, G), jnp.bfloat16),
            pltpu.VMEM((Hkv, G, D), jnp.bfloat16),
            pltpu.VMEM((2, 2, B, Sk, Dh), jnp.bfloat16),
            pltpu.VMEM((Hkv, B, R, Dh), jnp.bfloat16),
            pltpu.VMEM((1, R, Sk), jnp.float32),
            pltpu.VMEM((1, R, 128), jnp.float32),
            pltpu.VMEM((1, Sq, G), jnp.bfloat16),
            pltpu.VMEM((1, Sq, G), jnp.bfloat16),
            pltpu.VMEM((B, Sq, D), jnp.float32),
            pltpu.VMEM((B, Sq, D), jnp.bfloat16),
            pltpu.SMEM((1,), jnp.int32),
            pltpu.SemaphoreType.DMA((3 + Hkv + 9,)),
        ],
        compiler_params=pltpu.CompilerParams(
            vmem_limit_bytes=100 * 1024 * 1024,
            disable_bounds_checks=True,
            disable_semaphore_checks=True,
        ),
    )(x.reshape(B * Sq, D), k_cache, v_cache, wq, wo)
```

```python
import functools
import math

import jax
import jax.numpy as jnp
from jax import lax
import jax.experimental.pallas as pl
import jax.experimental.pallas.tpu as pltpu

HQ = 32
DH = 128
TK = 512
XB0 = 2
NLQ = 2
X1N = 3
X1Q = 2


def _kernel(x_hbm, k_hbm, v_hbm, wq_hbm, wo_hbm, out_hbm,
            x_s, wq_s, wo_s, kv_s, q_all, s_scr, m_scr, o_scr, o2_scr, acc_scr, out_s, z_ref,
            sems, *, B, Sq, rep, Hkv, Sk):
    scale = (DH ** -0.5) * math.log2(math.e)
    R = rep * Sq
    nC = Sk // TK
    nt = TK // 128
    G = rep * DH

    def mult(v, m):
        return v * m if isinstance(v, int) else pl.multiple_of(v * m, m)

    def kv_sem(slot):
        return sems.at[slot]

    wo_sem = sems.at[2]
    next_sem = [3 + Hkv]

    def new_sem():
        s = sems.at[next_sem[0]]
        next_sem[0] += 1
        return s

    def k_copy(g, sem, b0=0, n=B):
        return pltpu.make_async_copy(k_hbm.at[pl.ds(b0, n), g], kv_s.at[g & 1, 0, pl.ds(b0, n)], sem)

    def v_copy(g, sem, b0=0, n=B - 1):
        return pltpu.make_async_copy(v_hbm.at[pl.ds(b0, n), g], kv_s.at[g & 1, 1, pl.ds(b0 + 1, n)], sem)

    def vlast_copy(g, sem):
        return pltpu.make_async_copy(v_hbm.at[B - 1, g], kv_s.at[(g + 1) & 1, 1, 0], sem)

    def wq_copy(g):
        return pltpu.make_async_copy(wq_hbm.at[:, pl.ds(mult(g, G), G)], wq_s.at[g], sems.at[3 + g])

    def wo_copy(g, sem):
        return pltpu.make_async_copy(wo_hbm.at[pl.ds(mult(g, G), G), :], wo_s.at[g], sem)

    def x_copy(b0, n):
        rows = pl.ds(b0 * Sq, n * Sq)
        return pltpu.make_async_copy(x_hbm.at[rows], x_s.at[rows], new_sem())

    def out_copy(b0, n):
        return pltpu.make_async_copy(out_s.at[pl.ds(b0, n)], out_hbm.at[pl.ds(b0, n)], new_sem())

    def qproj(g, b0=0, nb=B):
        q = jnp.dot(x_s[b0 * Sq:(b0 + nb) * Sq, :], wq_s[g], preferred_element_type=jnp.float32)
        q = q.astype(jnp.bfloat16)
        for u in range(nb):
            for h in range(rep):
                q_all[g, b0 + u, h * Sq:(h + 1) * Sq, :] = q[u * Sq:(u + 1) * Sq, h * DH:(h + 1) * DH]

    def qk(g, b, fin=None):
        q = q_all[g, b]
        slot = g & 1
        pmx = None
        for j in range(nC):
            s = lax.dot_general(q, kv_s[slot, 0, b, j * TK:(j + 1) * TK, :], (((1,), (1,)), ((), ())),
                                preferred_element_type=jnp.float32) * scale
            s_scr[0, :, j * TK:(j + 1) * TK] = s
            if j == 0 and fin is not None:
                fin(s[:, 0:128])
            pm = s[:, 0:128]
            for t in range(1, nt):
                pm = jnp.maximum(pm, s[:, t * 128:(t + 1) * 128])
            pmx = pm if pmx is None else jnp.maximum(pmx, pm)
        m_scr[0] = jnp.broadcast_to(jnp.max(pmx, axis=-1, keepdims=True), (R, 128))

    def pv(slot, j0, tie=True, h0=0, nh=rep, o_dst=o_scr):
        z = z_ref[0]
        rows = slice(h0 * Sq, (h0 + nh) * Sq)
        m = m_scr[z, rows, :]
        p = jnp.exp2(s_scr[z, rows, :] - jnp.concatenate([m] * (Sk // 128), axis=1))
        lp = None
        for j in range(nC):
            ps = p[:, j * TK:j * TK + 128]
            for t in range(1, nt):
                ps = ps + p[:, j * TK + t * 128:j * TK + (t + 1) * 128]
            lp = ps if lp is None else lp + ps
        acc = jnp.dot(p.astype(jnp.bfloat16), kv_s[slot, 1, j0], preferred_element_type=jnp.float32)

        def fin(tie_v):
            lq = lp if tie_v is None else jnp.where(z != 0, tie_v, lp)
            l = jnp.sum(lq, axis=-1, keepdims=True)
            r = pl.reciprocal(l, approx=True)
            r = r * (2.0 - l * r)
            o = (acc * r).astype(jnp.bfloat16)
            for h in range(nh):
                o_dst[0, :, (h0 + h) * DH:(h0 + h + 1) * DH] = o[h * Sq:(h + 1) * Sq, :]

        if tie:
            return fin
        fin(None)

    def oproj(g, b, maybe_first=False):
        y = jnp.dot(o_scr[z_ref[0]], wo_s[g], preferred_element_type=jnp.float32)
        static = isinstance(g, int)
        if static:
            if g > 0:
                y = y + acc_scr[b]
        elif maybe_first:
            y = y + jnp.where(g > 0, acc_scr[b], 0.0)
        else:
            y = y + acc_scr[b]
        acc_scr[b] = y
        if not static and not maybe_first:
            out_s[b] = y.astype(out_s.dtype)

    def zstep(g, b):
        qk(g, b, pv(g & 1, b))
        if b == 0:
            oproj(g - 1, B - 1, maybe_first=True)
        else:
            oproj(g, b - 1)

    def whole(_, carry0):
        next_sem[0] = 3 + Hkv
        g1 = 1 + 2 * NLQ
        g2 = g1 + X1Q
        xa = x_copy(0, XB0)
        xb = x_copy(XB0, B - XB0)
        k0a = k_copy(0, new_sem(), 0, X1N)
        v0a = v_copy(0, new_sem(), 0, X1N - 1)
        wo0 = wo_copy(0, new_sem())
        v0b = v_copy(0, new_sem(), X1N - 1, B - X1N)
        k0b = k_copy(0, new_sem(), X1N, B - X1N)
        order = ([xa, wq_copy(0), xb] + [wq_copy(g) for g in range(1, g2)] + [k0a, v0a, wo0]
                 + [wq_copy(g) for g in range(g2, Hkv)] + [v0b, k0b]
                 + [vlast_copy(0, kv_sem(1)), k_copy(1, kv_sem(1)), v_copy(1, kv_sem(1)),
                    wo_copy(1, wo_sem)])
        for c in order:
            c.start()

        xa.wait()
        wq_copy(0).wait()
        qproj(0, 0, XB0)
        xb.wait()
        qproj(0, XB0, B - XB0)

        def qbody(j, carry):
            g = 2 * j + 1
            wq_copy(g).wait()
            wq_copy(g + 1).wait()
            qproj(g)
            qproj(g + 1)
            return carry

        lax.fori_loop(0, NLQ, qbody, 0)

        for c in [wq_copy(g) for g in range(g1, g2)] + [k0a, v0a, wo0]:
            c.wait()
        qk(0, 0)
        for g in range(g1, g2):
            qproj(g)
        for b in range(1, X1N):
            zstep(0, b)
        for c in [wq_copy(g) for g in range(g2, Hkv)] + [v0b, k0b]:
            c.wait()
        for g in range(g2, Hkv):
            qproj(g)
        for b in range(X1N, B):
            zstep(0, b)

        def body(g, carry):
            slot = g & 1
            pltpu.make_async_copy(kv_s.at[slot], kv_s.at[slot], kv_sem(slot)).wait()
            wo_copy(g, wo_sem).wait()
            zstep(g, 0)
            vlast_copy(g, kv_sem(1 - slot)).start()

            @pl.when(g < Hkv - 1)
            def _():
                k_copy(g + 1, kv_sem(1 - slot)).start()
                v_copy(g + 1, kv_sem(1 - slot)).start()
                wo_copy(g + 1, wo_sem).start()

            for b in range(1, B):
                zstep(g, b)
            return carry

        lax.fori_loop(1, Hkv, body, 0)

        oa = out_copy(0, B - 1)
        ob = out_copy(B - 1, 1)
        oa.start()
        vlast_copy(Hkv - 1, kv_sem(Hkv & 1)).wait()
        hh = rep // 2
        pv(Hkv & 1, 0, False, 0, hh, o_scr)
        pv(Hkv & 1, 0, False, hh, rep - hh, o2_scr)
        z = z_ref[0]
        y = acc_scr[B - 1] + jnp.dot(o_scr[z, :, :hh * DH], wo_s[Hkv - 1, :hh * DH, :],
                                     preferred_element_type=jnp.float32)
        y = y + jnp.dot(o2_scr[z, :, hh * DH:], wo_s[Hkv - 1, hh * DH:, :],
                        preferred_element_type=jnp.float32)
        out_s[B - 1] = y.astype(out_s.dtype)
        ob.start()
        oa.wait()
        ob.wait()
        return carry0

    z_ref[0] = 0
    lax.fori_loop(0, 1 + z_ref[0], whole, 0)


@jax.jit
def pallas_standalone__gqa_block_cached__near_ridge_kernel(x, k_cache, v_cache, wq, wo):
    B, Sq, D = x.shape
    _, Hkv, Sk, Dh = k_cache.shape
    rep = HQ // Hkv
    G = rep * Dh
    R = rep * Sq
    assert Dh == DH and Sk % TK == 0 and Sq % 16 == 0 and 1 + 2 * NLQ + X1Q <= Hkv and X1N < B
    kern = functools.partial(_kernel, B=B, Sq=Sq, rep=rep, Hkv=Hkv, Sk=Sk)
    any_spec = pl.BlockSpec(memory_space=pl.ANY)
    return pl.pallas_call(
        kern,
        in_specs=[any_spec] * 5,
        out_specs=any_spec,
        out_shape=jax.ShapeDtypeStruct((B, Sq, D), x.dtype),
        scratch_shapes=[
            pltpu.VMEM((B * Sq, D), jnp.bfloat16),
            pltpu.VMEM((Hkv, D, G), jnp.bfloat16),
            pltpu.VMEM((Hkv, G, D), jnp.bfloat16),
            pltpu.VMEM((2, 2, B, Sk, Dh), jnp.bfloat16),
            pltpu.VMEM((Hkv, B, R, Dh), jnp.bfloat16),
            pltpu.VMEM((1, R, Sk), jnp.float32),
            pltpu.VMEM((1, R, 128), jnp.float32),
            pltpu.VMEM((1, Sq, G), jnp.bfloat16),
            pltpu.VMEM((1, Sq, G), jnp.bfloat16),
            pltpu.VMEM((B, Sq, D), jnp.float32),
            pltpu.VMEM((B, Sq, D), jnp.bfloat16),
            pltpu.SMEM((1,), jnp.int32),
            pltpu.SemaphoreType.DMA((3 + Hkv + 9,)),
        ],
        compiler_params=pltpu.CompilerParams(
            vmem_limit_bytes=100 * 1024 * 1024,
            disable_bounds_checks=True,
            disable_semaphore_checks=True,
        ),
    )(x.reshape(B * Sq, D), k_cache, v_cache, wq, wo)
```
